```python
import jax
import jax.numpy as jnp

def _softmax(x, axis=-1):
    return jax.nn.softmax(x, axis=axis)
def _gelu(x):
    return jax.nn.gelu(x, approximate=True)
def _silu(x):
    return jax.nn.silu(x)
def _sigmoid(x):
    return jax.nn.sigmoid(x)
def _layernorm(x, axis=-1, eps=1e-5):
    m = jnp.mean(x, axis=axis, keepdims=True)
    v = jnp.var(x, axis=axis, keepdims=True)
    return (x - m) / jnp.sqrt(v + eps)
def _scatter_add(tgt, idx, src, axis=0):
    return tgt.at[idx].add(src)
def _segment_sum(src, seg, n):
    return jax.ops.segment_sum(src, seg, n)
class _Rng:
    def __init__(self, key):
        self._k = key
    def _next(self):
        self._k, sub = jax.random.split(self._k)
        return sub
    def normal(self, shape):
        return jax.random.normal(self._next(), shape, dtype=jnp.bfloat16)
    def randint(self, lo, hi, shape):
        return jax.random.randint(self._next(), shape, lo, hi, dtype=jnp.int32)
    def uniform(self, shape, lo=0.0, hi=1.0):
        return jax.random.uniform(self._next(), shape, jnp.bfloat16, lo, hi)
    def permutation(self, n):
        return jax.random.permutation(self._next(), n)


kernel_name = 'gated_mix__sliding_local_dilated__moe_arch_mod__prompt'

def setup_inputs():
    _rng = _Rng(jax.random.key(int.from_bytes(__import__("os").urandom(4), "little")))
    _w = (lambda a: (lambda t: t.astype(jnp.bfloat16) if jnp.issubdtype(t.dtype, jnp.floating) else t)(jnp.asarray(a)))
    def _A_setup():
        B, S, D = 1, 2048, 640
        return {
            "x": _w((lambda *s: _rng.normal(s) * 0.05)(B, S, D)),
            "wqkv": _w((lambda *s: _rng.normal(s) * 0.05)(D, 3 * D)),
            "wo": _w((lambda *s: _rng.normal(s) * 0.05)(D, D)),
        }
    _A_in = _A_setup()

    def _B_setup():
        B, S, D, F, C = 1, 2048, 640, 1728, 2
        return {
            "x": _w((lambda *s: _rng.normal(s) * 0.05)(B, S, D)),
            "w_r": _w((lambda *s: _rng.normal(s) * 0.05)(D)),
            "w_gate": _w((lambda *s: _rng.normal(s) * 0.05)(D, F)),
            "w_up": _w((lambda *s: _rng.normal(s) * 0.05)(D, F)),
            "w_down": _w((lambda *s: _rng.normal(s) * 0.05)(F, D)),
        }
    _B_in = _B_setup()

    return {
        "A_x": _A_in["x"],
        "A_wqkv": _A_in["wqkv"],
        "A_wo": _A_in["wo"],
        "B_x": _B_in["x"],
        "B_w_r": _B_in["w_r"],
        "B_w_gate": _B_in["w_gate"],
        "B_w_up": _B_in["w_up"],
        "B_w_down": _B_in["w_down"],
        "gate_w": _w((lambda *s: _rng.normal(s) * 0.05)(640)),
    }

def reference(A_x, A_wqkv, A_wo, B_x, B_w_r, B_w_gate, B_w_up, B_w_down, gate_w):
    def _A_ref(x, wqkv, wo):
        B, S, D = x.shape
        H = 32; Dh = D // H
        W, dil = 8, 2
        qkv = (lambda x, *d: x.transpose(*d))((x @ wqkv).reshape(B, S, 3, H, Dh), 2, 0, 3, 1, 4)
        q, k, v = qkv[0], qkv[1], qkv[2]
        scale = Dh ** -0.5
        pos = jnp.arange(S)
        off = jnp.arange(W) * dil
        idx = pos[:, None] - off[None, :]
        mask = idx >= 0
        idx_c = jnp.where(mask, idx, 0).reshape(-1)
        kg = k[:, :, idx_c, :].reshape(B, H, S, W, Dh)
        vg = v[:, :, idx_c, :].reshape(B, H, S, W, Dh)
        logits = jnp.einsum("bhsd,bhswd->bhsw", q, kg) * scale
        logits = jnp.where(mask[None, None, :, :], logits, -1e9)
        attn = _softmax(logits, axis=-1)
        o = jnp.einsum("bhsw,bhswd->bhsd", attn, vg)
        return (lambda x, *d: x.transpose(*d))(o, 0, 2, 1, 3).reshape(B, S, D) @ wo

    def _B_ref(x, w_r, w_gate, w_up, w_down):
        B, S, D = x.shape
        C = 2
        r = x @ w_r
        idx = jnp.argsort(-r, axis=-1)[:, :C]
        idx_e = jnp.repeat(idx.reshape(B, C, 1), D, axis=2)
        x_sel = jnp.take_along_axis(x, idx_e, axis=1)
        g = _silu(x_sel @ w_gate)
        u = x_sel @ w_up
        y = (g * u) @ w_down
        r_sel = _sigmoid(jnp.take_along_axis(r, idx, axis=1))
        y = y * r_sel.reshape(B, C, 1)
        b_off = (jnp.arange(B) * S).reshape(B, 1)
        flat_idx = (idx + b_off).reshape(B * C)
        zero = (x * 0.0).reshape(B * S, D)
        upd = _scatter_add(zero, flat_idx, y.reshape(B * C, D), axis=0)
        return x + upd.reshape(B, S, D)

    x = A_x
    g = _sigmoid((x * gate_w).sum(-1, keepdims=True))
    a = _A_ref(x, A_wqkv, A_wo)
    b = _B_ref(x, B_w_r, B_w_gate, B_w_up, B_w_down)
    return g * a + (1 - g) * b
```

```python
import functools
import numpy as np
import jax
import jax.numpy as jnp
import jax.experimental.pallas as pl
import jax.experimental.pallas.tpu as pltpu

S, D, F = 2048, 640, 1728
H, DH, W, DIL, CAP = 32, 20, 8, 2, 2
NJ = D // 128
HALO = 16
LOG2E = 1.4426950408889634
F32, BF16, U32 = jnp.float32, jnp.bfloat16, jnp.uint32
NT_DIMS = (((1,), (1,)), ((), ()))


def _iota(shape, dim):
    return jax.lax.broadcasted_iota(jnp.int32, shape, dim)


def make(T=256, order="AAACAACAACACCCCC", ffn_at=72, ffn_every=1, r_from=26, r_every=1, x_at=25, x_span=18, glag=3, lag=1, do_ffn=True, do_attn=True,
         NW=1, qtie=2, smtie=0, WC=320, hold=(1, 6), split_out=1, prof=0, tr=0, fstart=4, abl='', RB=32, pvlag=2, dep=True, b_end=None, vfirst=False, flags=None):
    NT = S // T
    G = T // 16
    NWC = D // WC

    def kernel(x_hbm, wqkv_hbm, wo_hbm, wr_hbm, wg_hbm, wu_hbm, wd_hbm, gw_hbm, out_hbm,
               big, w_v, wo_v, wo_f, xu, wu32, q_s, k_s, v_s, o_s, g_s, out_v, wr_v, gw_v, sem, wsem, osem):
        x_v = big.at[pl.ds(0, S)]
        wg_v, wu_v, wd_v = (big.at[pl.ds(S + n * F, F)] for n in range(3))
        x_cp = [pltpu.make_async_copy(x_hbm.at[0, pl.ds(a, n)], x_v.at[pl.ds(a, n)], sem.at[i])
                for i, (a, n) in enumerate(((0, T), (T, T), (2 * T, S - 2 * T)))]
        wk_cp = [pltpu.make_async_copy(wqkv_hbm.at[pl.ds(WC * c, WC), pl.ds(D, D)], w_v.at[1, pl.ds(WC * c, WC)], wsem.at[c]) for c in range(NWC)]
        w_cp = [pltpu.make_async_copy(wqkv_hbm.at[:, pl.ds(p * D, D)], w_v.at[p], sem.at[NT + p]) for p in (0, 2)]
        wo_cp = pltpu.make_async_copy(wo_hbm, wo_v, sem.at[NT + 3])
        wg_cp = pltpu.make_async_copy(wg_hbm, wg_v, sem.at[NT + 4])
        wu_cp = pltpu.make_async_copy(wu_hbm, wu_v, sem.at[NT + 5])
        wd_cp = pltpu.make_async_copy(wd_hbm, wd_v, sem.at[NT + 6])
        wr_cp = pltpu.make_async_copy(wr_hbm, wr_v, sem.at[NT + 7])
        gw_cp = pltpu.make_async_copy(gw_hbm, gw_v, sem.at[NT + 8])
        o_cp = [pltpu.make_async_copy(out_v.at[pl.ds(i * T, T)], out_hbm.at[0, pl.ds(i * T, T)], osem.at[i, 0]) for i in range(NT)]

        def o_col(i, j):
            return pltpu.make_async_copy(out_v.at[pl.ds(i * T, T), pl.ds(128 * j, 128)], out_hbm.at[0, pl.ds(i * T, T), pl.ds(128 * j, 128)], osem.at[i, j])

        lane = _iota((8, 128), 1)
        st = dict(racc=[jnp.zeros((8, 128), F32) for _ in range(S // 1024)], y=None, hh={}, dep={}, res={}, n=-1, slot=0, true=None)

        def add_dep(*vals):
            k = st["slot"]
            for v in vals:
                v = pltpu.bitcast(v, U32)
                st["dep"][k] = v if st["dep"].get(k) is None else st["dep"][k] | v

        def tie(lhs):
            d, st["dep"] = st["dep"], {}
            if not d or not dep:
                return lhs
            top = [lhs[tr:tr + 8, 128 * k:128 * (k + 1)] for k in range(NJ)]
            top = [jnp.where(st["true"], t, d[k]) if k in d else t for k, t in enumerate(top)]
            parts = [lhs[:tr]] if tr else []
            return jnp.concatenate(parts + [jnp.concatenate(top, axis=1), lhs[tr + 8:]], axis=0)

        def permute_w(p, r):
            src = [pltpu.bitcast(w_v[p, pl.ds(16 * r, 16), pl.ds(128 * t, 128)], U32) for t in range(NJ)]
            for j in range(NJ):
                m = src[0]
                for t in range(1, NJ):
                    m = jnp.where((128 * t + lane) % 5 == j, src[t], m)
                m = jnp.take_along_axis(m, (20 * (lane % 32) + 5 * (lane // 32) + j) % 128, axis=1)
                wu32[p, pl.ds(8 * r, 8), pl.ds(128 * j, 128)] = m

        def widen_wo(t, c):
            blk = wo_v[pl.ds(64 * c, 64), pl.ds(128 * t, 128)].astype(F32)
            wo_f[t, pl.ds(64 * c, 64), :] = blk
            add_dep(blk[56:])

        def permute_wo(t, j):
            for a in range(4):
                blk = pltpu.bitcast(wo_f[t, pl.ds(5 * a + j, 32, stride=20), :].astype(BF16), U32)
                wu32[3, pl.ds(64 * j + 16 * a, 16), pl.ds(128 * t, 128)] = blk
            add_dep(blk[8:])

        def pack_x(i, b):
            r0 = i * T + 16 * b
            blk = pltpu.bitcast(x_v[pl.ds(r0, 16), :], U32)
            xu[pl.ds(r0 // 2, 8), :] = blk
            add_dep(blk[:, D - 128:])

        def proj(i, p, j0, nw):
            dst, off = ((q_s, 0), (k_s, HALO), (v_s, HALO))[p]
            lhs = pltpu.bitcast(tie(xu[pl.ds(i * T // 2, T // 2), :]), BF16)
            rhs = pltpu.bitcast(wu32[p, :, pl.ds(128 * j0, 128 * nw)], BF16)
            r = jnp.dot(lhs, rhs, preferred_element_type=F32)
            st["res"][st["n"]] = [r[z:z + 8, :128] for z in range(0, T, T // 4)]
            if i == 0 and st["n"] in hold:
                w_v[3, pl.ds(0, 16), pl.ds(0, 128)] = r[:16, :128].astype(BF16)
            for j in range(nw):
                dst[j0 + j, pl.ds(off + i * T, T), :] = r[:, 128 * j:128 * (j + 1)]
                if i == 0 and p == 2:
                    v_s[j0 + j, pl.ds(0, HALO), :] = jnp.broadcast_to(r[0:1, 128 * j:128 * (j + 1)], (HALO, 128))

        sub = _iota((8, 128), 0)

        def router(i):
            if "wrg" not in st:
                wr = jnp.broadcast_to(wr_v[...].astype(F32).reshape(1, D), (8, D))
                gw = jnp.broadcast_to(gw_v[...].astype(F32).reshape(1, D), (8, D))
                st["wrg"] = jnp.concatenate([wr, gw], axis=0).astype(BF16)
            xt = pltpu.bitcast(xu[pl.ds(64 * i, 64), :], BF16)
            rg = jax.lax.dot_general(st["wrg"], xt, NT_DIMS, preferred_element_type=F32)
            st["racc"][i // 8] = jnp.where(sub == i % 8, rg[:8], st["racc"][i // 8])
            st["g", i] = jax.nn.sigmoid(rg[8:])

        def gate(i):
            diag = [jnp.where(lane == sub + 8 * u, st["g", n], 0.0)
                    for n in range(i * T // 128, (i + 1) * T // 128) for u in range(16)]
            diag = jnp.concatenate(diag, axis=0).astype(BF16)
            g_s[pl.ds(i * T, T), :] = jnp.dot(diag, jnp.ones((128, 128), BF16), preferred_element_type=F32)

        cs = (DH ** -0.5) * LOG2E

        rmat = jnp.where(_iota((128, 128), 0) % 32 == _iota((128, 128), 1) % 32, 1.0, 0.0).astype(BF16)

        def qk(i, b):
            r0 = i * T + RB * b
            parts = [[None] * (RB // 8) for _ in range(W)]
            for u in range(RB // 8):
                q = [q_s[j, pl.ds(r0 + 8 * u, 8), :] for j in range(NJ)]
                if qtie and st["n"] + 1 - qtie in st["res"]:
                    rs = st["res"][st["n"] + 1 - qtie]
                    q = [jnp.where(st["true"], qq, rs[u * len(rs) // (RB // 8)]) for qq in q]
                for w in range(W):
                    s = None
                    for j in range(NJ):
                        t = q[j] * k_s[j, pl.ds(HALO + r0 + 8 * u - DIL * w, 8), :]
                        s = t if s is None else s + t
                    parts[w][u] = s
            cat = jnp.concatenate([p for pw in parts for p in pw], axis=0).astype(BF16)
            st["l", i, b] = jnp.dot(cat, rmat, preferred_element_type=F32)

        def probs(i, b, u):
            if ("p", i, b, u) not in st:
                lg = st["l", i, b]
                r0 = i * T + RB * b + 8 * u
                ls = []
                csv = cs
                if smtie and st["n"] + 1 - smtie in st["res"]:
                    rs = st["res"][st["n"] + 1 - smtie]
                    csv = jnp.where(st["true"], cs, rs[min(3, st["slot"])])
                for w in range(W):
                    s = lg[w * RB + 8 * u:w * RB + 8 * u + 8] * csv
                    if r0 < DIL * w:
                        s = jnp.where(_iota((8, 128), 0) + r0 >= DIL * w, s, -1e9 * LOG2E)
                    ls.append(s)
                m = functools.reduce(jnp.maximum, ls)
                ps = [jnp.exp2(l - m) for l in ls]
                st["p", i, b, u] = (ps, 1.0 / functools.reduce(lambda a, b: a + b, ps))
            return st["p", i, b, u]

        def pv(i, b, u2, j):
            halves = []
            for u in (2 * u2, 2 * u2 + 1):
                r0 = i * T + RB * b + 8 * u
                ps, inv = probs(i, b, u)
                o = None
                for w in range(W):
                    t = ps[w] * v_s[j, pl.ds(HALO + r0 - DIL * w, 8), :]
                    o = t if o is None else o + t
                halves.append(o * inv)
            r0 = i * T + RB * b + 16 * u2
            o = jnp.concatenate(halves, axis=0).astype(BF16)
            o_s[pl.ds(r0 // 2, 8), pl.ds(128 * j, 128)] = pltpu.bitcast(o, U32)
            add_dep(o)

        def outproj(i, j0, nw):
            lhs = pltpu.bitcast(tie(o_s[pl.ds(i * T // 2, T // 2), :]), BF16)
            rhs = pltpu.bitcast(wu32[3, :, pl.ds(128 * j0, 128 * nw)], BF16)
            a = jnp.dot(lhs, rhs, preferred_element_type=F32)
            st["res"][st["n"]] = [a[z:z + 8, :128] for z in range(0, T, T // 4)]
            g = g_s[pl.ds(i * T, T), :]
            for j in range(nw):
                cols = pl.ds(128 * (j0 + j), 128)
                xj = pltpu.bitcast(xu[pl.ds(i * T // 2, T // 2), cols], BF16).astype(F32)
                if 'm' in abl:
                    out_v[pl.ds(i * T, T), cols] = a[:, 128 * j:128 * (j + 1)].astype(BF16)
                    continue
                out_v[pl.ds(i * T, T), cols] = (xj + g * (a[:, 128 * j:128 * (j + 1)] - xj)).astype(BF16)

        def top2():
            racc = st["racc"]
            tok = [(sub + 8 * c) * 128 + lane for c in range(len(racc))]
            rb = [r.astype(BF16).astype(F32) for r in racc]
            rb = [jnp.where(r != r, -jnp.inf, r) for r in rb]
            taken = [t < 0 for t in tok]
            sel = []
            row16 = _iota((16, D), 0)
            xs = jnp.zeros((16, D), F32)
            for n in range(CAP):
                m = functools.reduce(jnp.maximum, [jnp.where(tk, -jnp.inf, r) for r, tk in zip(rb, taken)])
                m = jnp.max(jnp.max(m, axis=1, keepdims=True), axis=0, keepdims=True)
                c = functools.reduce(jnp.minimum, [jnp.where((r == m) & jnp.logical_not(tk), t, S) for r, t, tk in zip(rb, tok, taken)])
                c = jnp.min(jnp.min(c.astype(F32), axis=1, keepdims=True), axis=0, keepdims=True).astype(jnp.int32)
                taken = [tk | (t == c) for t, tk in zip(tok, taken)]
                idx = c[0, 0]
                sel.append((idx, m))
                base = pl.multiple_of(jnp.clip((idx // 16) * 16, 0, S - 16), 16)
                blk = x_v[pl.ds(base, 16), :].astype(F32)
                xr = jnp.sum(jnp.where(row16 + base == idx, blk, 0.0), axis=0, keepdims=True)
                xs = jnp.where(row16 == n, xr, xs)
            st["sel"] = sel
            st["xs"] = xs.astype(BF16)

        def ffn_piece(kind, n):
            f0 = 128 * n
            fn_ = min(128, F - f0)
            if kind == 0:
                st["hg"] = jax.lax.dot_general(st["xs"], wg_v[pl.ds(f0, fn_), :], NT_DIMS, preferred_element_type=F32)
            elif kind == 1:
                hu = jax.lax.dot_general(st["xs"], wu_v[pl.ds(f0, fn_), :], NT_DIMS, preferred_element_type=F32)
                hg = st["hg"]
                st["hh"][n] = (hg * jax.nn.sigmoid(hg) * hu).astype(BF16)
            else:
                y = jnp.dot(st["hh"][n], wd_v[pl.ds(f0, fn_), :], preferred_element_type=F32)
                st["y"] = y if st["y"] is None else st["y"] + y

        def patch(lo, hi, js=range(NJ)):
            row16 = _iota((16, 128), 0)
            for n, (idx, m) in enumerate(st["sel"]):
                yn = st["y"][n:n + 1] * jax.nn.sigmoid(m)
                base = pl.multiple_of(jnp.clip((idx // 16) * 16, lo, hi - 16), 16)
                og = 1.0 - g_s[pl.ds(base, 16), :]
                hit = row16 + base == idx
                for j in js:
                    cur = out_v[pl.ds(base, 16), pl.ds(128 * j, 128)].astype(F32)
                    new = jnp.where(hit, cur + og * yn[:, 128 * j:128 * (j + 1)], cur)
                    out_v[pl.ds(base, 16), pl.ds(128 * j, 128)] = new.astype(BF16)

        groups = [(j0, min(NW, NJ - j0)) for j0 in range(0, NJ, NW)]
        mxu = []
        na = nc = 0
        for ch in order:
            if ch == "A":
                mxu += [("A", na, p, j0, nw) for p in (1, 2, 0) for j0, nw in groups]
                na += 1
            else:
                mxu += [("C", nc, 3, j0, nw) for j0, nw in groups]
                nc += 1
        assert na == NT and nc == NT
        pos, t = [], 0
        for m_ in mxu:
            pos.append(t)
            t += m_[4]
        total = t
        a_done = {i: max(pos[n] + m_[4] for n, m_ in enumerate(mxu) if m_[0] == "A" and m_[1] == i) for i in range(NT)}
        c_start = {i: min(pos[n] for n, m_ in enumerate(mxu) if m_[0] == "C" and m_[1] == i) for i in range(NT)}
        b0 = a_done[0]
        b1 = c_start[NT - 1] if b_end is None else b_end
        vq = []

        def xdue(i, b):
            if i == 0:
                return 0
            if i == 1:
                return 10 + 3.8 * b / G
            return x_at + x_span * ((i - 2) * G + b) / ((NT - 2) * G)

        for i in range(NT):
            for b in range(G):
                due = b0 + (b1 - b0) * (i * G + b) / (NT * G)
                due = min(max(due, a_done[i] + lag - 1), c_start[i])
                if do_attn and (16 * b) % RB == 0:
                    span = (b1 - b0) * RB / S
                    due = min(due, c_start[i] - pvlag - span)
                    vq.append((due, 1, ("QK", i, 16 * b // RB)))
                    nsub = (RB // 16) * (NJ + 2)
                    for u2 in range(RB // 16):
                        for z in range(NJ + 2):
                            t_sub = due + pvlag + span * (u2 * (NJ + 2) + z) / nsub
                            if z < 2:
                                vq.append((t_sub, 0.5, ("SM", i, 16 * b // RB, 2 * u2 + z)))
                            else:
                                vq.append((t_sub, 0.5, ("PV", i, 16 * b // RB, u2, z - 2)))
                if i >= 1:
                    vq.append((xdue(i, b), -1, ("X", i, b)))
            vq.append((c_start[i] - glag, 0, ("G", i)))
        for n in range(S // 128):
            i = n * 128 // T
            vq.append((max(r_from + n * r_every, np.ceil(xdue(i, G - 1)) + 1), 0, ("R", n)))
        r_to = max(e[0] for e in vq if e[2][0] == "R")
        for r in range(D // 16):
            vq.append((hold[0] + 0.5 + r / 1000, -2, ("W", 2, r)))
            vq.append((hold[1] + 0.5 + r / 1000, -2, ("W", 0, r)))
        wo_at = c_start[0] - 16
        for t_ in range(NJ):
            for c in range(D // 64):
                vq.append((wo_at + (t_ * 10 + c) / NJ, -2, ("WF", t_, c)))
            for j in range(NJ):
                vq.append((wo_at + 10.2 + t_ + j / NJ, -2, ("WO", t_, j)))
        if do_ffn:
            vq.append((r_to + 2, 2, ("T",)))
            nf = -(-F // 128)
            seq = []
            for n in range(nf):
                seq += [(0, n), (1, n)]
                if n >= 1:
                    seq.append((2, n - 1))
            seq.append((2, nf - 1))
            for n, kn in enumerate(seq):
                vq.append((ffn_at + n * ffn_every, 3, ("F",) + kn))
            ffn_done = ffn_at + len(seq) * ffn_every
        else:
            ffn_done = 0
        vq.sort(key=lambda e: (e[0], e[1]))

        waited = set()

        def need(name, cp):
            if name not in waited:
                waited.add(name)
                cp.wait()

        def emit(item):
            k = item[0]
            if k == "QK":
                qk(item[1], item[2])
            elif k == "PV":
                pv(*item[1:])
            elif k == "SM":
                add_dep(probs(*item[1:])[1])
            elif k == "R":
                need("wr", wr_cp); need("gw", gw_cp)
                if 'r' not in abl:
                    router(item[1])
            elif k == "G":
                gate(item[1])
            elif k == "X":
                if item[1] == 1:
                    need(("x", 1), x_cp[1])
                elif ("x", 2) not in waited:
                    need(("x", 2), x_cp[2]); need("wr", wr_cp); need("gw", gw_cp); need("wo", wo_cp)
                    wg_cp.start(); wu_cp.start(); wd_cp.start()
                pack_x(item[1], item[2])
            elif k == "W":
                if item[1] == 1:
                    c = 16 * item[2] // WC
                    if ("wk", c) not in waited:
                        need(("wk", c), wk_cp[c])
                        if c == 0:
                            w_cp[0].start(); x_cp[1].start()
                elif ("w", item[1]) not in waited:
                    need(("w", item[1]), w_cp[item[1] // 2])
                    if item[1] == 2:
                        wr_cp.start(); gw_cp.start()
                        x_cp[2].start()
                        wo_cp.start()
                if 'w' not in abl:
                    permute_w(item[1], item[2])
            elif k == "WF":
                need("wo", wo_cp)
                widen_wo(item[1], item[2])
            elif k == "WO":
                permute_wo(item[1], item[2])
            elif k == "T":
                top2()
            elif k == "F":
                need("wg", wg_cp); need("wu", wu_cp); need("wd", wd_cp)
                ffn_piece(item[1], item[2])

        x_cp[0].start()
        for c in range(NWC):
            wk_cp[c].start()
        w_cp[1].start()
        for j in range(NJ):
            k_s[j, pl.ds(0, HALO), :] = jnp.zeros((HALO, 128), F32)
        need(("x", 0), x_cp[0])
        for b in range(G):
            pack_x(0, b)
        for r in range(D // 16):
            emit(("W", 1, r))
        st["dep"] = {}
        u0 = xu[pl.ds(0, 8), pl.ds(0, 128)]
        st["true"] = ((u0 & 1) + ((~u0) & 1)) == 1

        def soft(item, m_):
            return item[0] in ("SM", "PV", "WF", "WO", "X") and not (m_[0] == "C" and m_[1] == item[1])

        qi = 0
        sent = 0
        cdone = 0
        scope = None
        for n, m_ in enumerate(mxu):
            if prof and n % prof == 0:
                if scope is not None:
                    scope.__exit__(None, None, None)
                scope = jax.named_scope("u%03d" % n)
                scope.__enter__()
            while qi < len(vq) and vq[qi][0] <= pos[n] + (m_[4] * (NJ - 1) / NJ if soft(vq[qi][2], m_) else 0):
                st["slot"] = min(NJ - 1, max(0, int(np.ceil((vq[qi][0] - pos[n]) * NJ / m_[4] - 1e-9))))
                emit(vq[qi][2]); qi += 1
            st["n"] = n
            if m_[0] == "A":
                proj(m_[1], m_[2], m_[3], m_[4])
            else:
                outproj(m_[1], m_[3], m_[4])
                if m_[1] >= NT - split_out:
                    assert sent == NT - split_out
                    js = range(m_[3], m_[3] + m_[4])
                    if do_ffn:
                        patch(m_[1] * T, m_[1] * T + T, js)
                    for j in js:
                        o_col(m_[1], j).start()
                elif m_[3] + m_[4] == NJ:
                    cdone = m_[1] + 1
            if cdone > sent and pos[n] >= ffn_done:
                if do_ffn:
                    patch(sent * T, cdone * T)
                for i in range(sent, cdone):
                    o_cp[i].start()
                sent = cdone
        assert qi == len(vq)
        if scope is not None:
            scope.__exit__(None, None, None)
        if not do_ffn and 'f' not in abl:
            wg_cp.wait(); wu_cp.wait(); wd_cp.wait()
        for i in range(NT - split_out):
            o_cp[i].wait()
        for i in range(NT - split_out, NT):
            for j in range(NJ):
                o_col(i, j).wait()

    hbm = pl.BlockSpec(memory_space=pltpu.HBM)

    @jax.jit
    def fn(A_x, A_wqkv, A_wo, B_x, B_w_r, B_w_gate, B_w_up, B_w_down, gate_w):
        return pl.pallas_call(
            kernel,
            out_shape=jax.ShapeDtypeStruct((1, S, D), BF16),
            in_specs=[hbm] * 8,
            out_specs=hbm,
            scratch_shapes=[
                pltpu.VMEM((S + 3 * F, D), BF16), pltpu.VMEM((4, D, D), BF16), pltpu.VMEM((D, D), BF16),
                pltpu.VMEM((NJ, D, 128), F32),
                pltpu.VMEM((S // 2, D), U32), pltpu.VMEM((4, D // 2, D), U32),
                pltpu.VMEM((NJ, S, 128), F32), pltpu.VMEM((NJ, S + HALO, 128), F32), pltpu.VMEM((NJ, S + HALO, 128), F32),
                pltpu.VMEM((S // 2, D), U32), pltpu.VMEM((S, 128), F32), pltpu.VMEM((S, D), BF16),
                pltpu.VMEM((D,), BF16), pltpu.VMEM((D,), BF16),
                pltpu.SemaphoreType.DMA((NT + 9,)), pltpu.SemaphoreType.DMA((NWC,)), pltpu.SemaphoreType.DMA((NT, NJ)),
            ],
            compiler_params=pltpu.CompilerParams(vmem_limit_bytes=100 * 1024 * 1024, flags=flags),
        )(A_x, A_wqkv, A_wo, B_w_r, B_w_gate.T, B_w_up.T, B_w_down, gate_w)
    return fn


_fn = make()


@jax.jit
def pallas_gated_mix__sliding_local_dilated__moe_arch_mod__prompt_kernel(
    A_x, A_wqkv, A_wo, B_x, B_w_r, B_w_gate, B_w_up, B_w_down, gate_w):
    return _fn(A_x, A_wqkv, A_wo, B_x, B_w_r, B_w_gate, B_w_up, B_w_down, gate_w)
```

```python
import functools
import numpy as np
import jax
import jax.numpy as jnp
import jax.experimental.pallas as pl
import jax.experimental.pallas.tpu as pltpu

S, D, F = 2048, 640, 1728
H, DH, W, DIL, CAP = 32, 20, 8, 2, 2
NJ = D // 128
HALO = 16
LOG2E = 1.4426950408889634
F32, BF16, U32 = jnp.float32, jnp.bfloat16, jnp.uint32
NT_DIMS = (((1,), (1,)), ((), ()))


def _iota(shape, dim):
    return jax.lax.broadcasted_iota(jnp.int32, shape, dim)


def make(T=256, order="AAAACACAACACCCCC", ffn_at=78, ffn_per=4, head='K0K1V0V1Q0Q1', r_from=17, r_every=3, x_at=38, x_span=28, glag=1, x1lag=1.1, wo_span=11, lag=1, do_ffn=True, do_attn=True,
         NW=1, qtie=2, WC=320, hold=(7, 15), row_cuts=(4, 5, 6, 7), col_cuts=(1, 2, 3, 4, 5), prof=0, tr=0, fstart=4, abl='', RB=16, pvlag=3, dep=True, b_end=None, vfirst=False, flags=None):
    NT = S // T
    G = T // 16
    NWC = D // WC

    def kernel(x_hbm, wqkv_hbm, wo_hbm, wr_hbm, wg_hbm, wu_hbm, wd_hbm, gw_hbm, out_hbm,
               big, w_v, wo_v, wo_f, xu, wu32, q_s, k_s, v_s, o_s, g_s, y_s, out_v, wr_v, gw_v, sem, wsem, osem):
        x_v = big.at[pl.ds(0, S)]
        wg_v, wu_v, wd_v = (big.at[pl.ds(S + n * F, F)] for n in range(3))
        x_cp = [pltpu.make_async_copy(x_hbm.at[0, pl.ds(a, n)], x_v.at[pl.ds(a, n)], sem.at[i])
                for i, (a, n) in enumerate(((0, T), (T, T), (2 * T, T), (3 * T, S - 3 * T)))]
        wk_cp = [pltpu.make_async_copy(wqkv_hbm.at[pl.ds(WC * c, WC), pl.ds(D, D)], w_v.at[1, pl.ds(WC * c, WC)], wsem.at[c]) for c in range(NWC)]
        w_cp = [pltpu.make_async_copy(wqkv_hbm.at[:, pl.ds(p * D, D)], w_v.at[p], sem.at[NT + p]) for p in (0, 2)]
        wo_cp = pltpu.make_async_copy(wo_hbm, wo_v, sem.at[NT + 3])
        wg_cp = pltpu.make_async_copy(wg_hbm, wg_v, sem.at[NT + 4])
        wu_cp = pltpu.make_async_copy(wu_hbm, wu_v, sem.at[NT + 5])
        wd_cp = pltpu.make_async_copy(wd_hbm, wd_v, sem.at[NT + 6])
        wr_cp = pltpu.make_async_copy(wr_hbm, wr_v, sem.at[NT + 7])
        gw_cp = pltpu.make_async_copy(gw_hbm, gw_v, sem.at[NT + 8])

        def o_copy(i0, i1, j0, j1, n):
            rows, cols = pl.ds(i0 * T, (i1 - i0) * T), pl.ds(128 * j0, 128 * (j1 - j0))
            return pltpu.make_async_copy(out_v.at[rows, cols], out_hbm.at[0, rows, cols], osem.at[n])

        lane = _iota((8, 128), 1)
        st = dict(racc=[jnp.zeros((8, 128), F32) for _ in range(S // 1024)], y=None, hh={}, dep={}, res={}, n=-1, slot=0, true=None)

        def add_dep(*vals):
            k = st["slot"]
            for v in vals:
                v = pltpu.bitcast(v, U32)
                st["dep"][k] = v if st["dep"].get(k) is None else st["dep"][k] | v

        def tie(lhs):
            d, st["dep"] = st["dep"], {}
            if not d or not dep:
                return lhs
            top = [lhs[tr:tr + 8, 128 * k:128 * (k + 1)] for k in range(NJ)]
            top = [jnp.where(st["true"], t, d[k]) if k in d else t for k, t in enumerate(top)]
            parts = [lhs[:tr]] if tr else []
            return jnp.concatenate(parts + [jnp.concatenate(top, axis=1), lhs[tr + 8:]], axis=0)

        def permute_w(p, r):
            src = [pltpu.bitcast(w_v[p, pl.ds(16 * r, 16), pl.ds(128 * t, 128)], U32) for t in range(NJ)]
            for j in range(NJ):
                m = src[0]
                for t in range(1, NJ):
                    m = jnp.where((128 * t + lane) % 5 == j, src[t], m)
                if j:
                    m = pltpu.roll(m, 128 - j, 1)
                wu32[p, pl.ds(8 * r, 8), pl.ds(128 * j, 128)] = m

        def widen_wo(t, c):
            blk = wo_v[pl.ds(64 * c, 64), pl.ds(128 * t, 128)].astype(F32)
            wo_f[t, pl.ds(64 * c, 64), :] = blk
            if c == 0:
                wo_f[t, pl.ds(D, 8), :] = jnp.zeros((8, 128), F32)
            add_dep(blk[56:])

        def permute_wo(t, j, c):
            outs = []
            for m0 in range(32 * c, 32 * c + 32, 8):
                tile = (3 * (_iota((8, 128), 0) + m0)) % 5
                blk = wo_f[t, pl.ds(m0 + j, 8), :]
                for z in range(1, NJ):
                    blk = jnp.where(tile == z, wo_f[t, pl.ds(128 * z + m0 + j, 8), :], blk)
                outs.append(blk)
            blk = pltpu.bitcast(jnp.concatenate(outs, axis=0).astype(BF16), U32)
            wu32[3, pl.ds(64 * j + 16 * c, 16), pl.ds(128 * t, 128)] = blk
            add_dep(blk[:8], blk[8:])

        def pack_x(i, b):
            r0 = i * T + 16 * b
            blk = pltpu.bitcast(x_v[pl.ds(r0, 16), :], U32)
            xu[pl.ds(r0 // 2, 8), :] = blk
            add_dep(blk[:, D - 128:])

        def proj(i, p, j0, nw):
            dst, off = ((q_s, 0), (k_s, HALO), (v_s, HALO))[p]
            lhs = pltpu.bitcast(tie(xu[pl.ds(i * T // 2, T // 2), :]), BF16)
            rhs = pltpu.bitcast(wu32[p, :, pl.ds(128 * j0, 128 * nw)], BF16)
            r = jnp.dot(lhs, rhs, preferred_element_type=F32)
            st["res"][st["n"]] = [r[z:z + 8, :128] for z in range(0, T, T // 4)]
            if st["n"] in hold:
                w_v[3, pl.ds(0, 16), pl.ds(0, 128)] = r[:16, :128].astype(BF16)
            for j in range(nw):
                dst[j0 + j, pl.ds(off + i * T, T), :] = r[:, 128 * j:128 * (j + 1)]
                if i == 0 and p == 2:
                    v_s[j0 + j, pl.ds(0, HALO), :] = jnp.broadcast_to(r[0:1, 128 * j:128 * (j + 1)], (HALO, 128))

        sub = _iota((8, 128), 0)

        def router(i):
            if "wrg" not in st:
                wr = jnp.broadcast_to(wr_v[...].astype(F32).reshape(1, D), (8, D))
                gw = jnp.broadcast_to(gw_v[...].astype(F32).reshape(1, D), (8, D))
                st["wrg"] = jnp.concatenate([wr, gw], axis=0).astype(BF16)
            xt = pltpu.bitcast(xu[pl.ds(64 * i, 64), :], BF16)
            rg = jax.lax.dot_general(st["wrg"], xt, NT_DIMS, preferred_element_type=F32)
            st["racc"][i // 8] = jnp.where(sub == i % 8, rg[:8], st["racc"][i // 8])
            st["g", i] = jax.nn.sigmoid(rg[8:])

        def gate(i):
            diag = [jnp.where(lane == sub + 8 * u, st["g", n], 0.0)
                    for n in range(i * T // 128, (i + 1) * T // 128) for u in range(16)]
            diag = jnp.concatenate(diag, axis=0).astype(BF16)
            g_s[pl.ds(i * T, T), :] = jnp.dot(diag, jnp.ones((128, 128), BF16), preferred_element_type=F32)

        cs = (DH ** -0.5) * LOG2E

        rmat = jnp.where((77 * _iota((128, 128), 0)) % 128 // 4 == (77 * _iota((128, 128), 1)) % 128 // 4, 1.0, 0.0).astype(BF16)

        def qk(i, b):
            r0 = i * T + RB * b
            parts = [[None] * (RB // 8) for _ in range(W)]
            for u in range(RB // 8):
                q = [q_s[j, pl.ds(r0 + 8 * u, 8), :] for j in range(NJ)]
                if qtie and st["n"] + 1 - qtie in st["res"]:
                    rs = st["res"][st["n"] + 1 - qtie]
                    csv = jnp.where(st["true"], cs, rs[u * len(rs) // (RB // 8)])
                else:
                    csv = cs
                q = [qq * csv for qq in q]
                for w in range(W):
                    s = None
                    for j in range(NJ):
                        t = q[j] * k_s[j, pl.ds(HALO + r0 + 8 * u - DIL * w, 8), :]
                        s = t if s is None else s + t
                    parts[w][u] = s
            cat = jnp.concatenate([p for pw in parts for p in pw], axis=0).astype(BF16)
            st["l", i, b] = jnp.dot(cat, rmat, preferred_element_type=F32)

        def probs(i, b, u):
            if ("p", i, b, u) not in st:
                lg = st["l", i, b]
                r0 = i * T + RB * b + 8 * u
                ls = []
                for w in range(W):
                    s = lg[w * RB + 8 * u:w * RB + 8 * u + 8]
                    if r0 < DIL * w:
                        s = jnp.where(_iota((8, 128), 0) + r0 >= DIL * w, s, -1e9 * LOG2E)
                    ls.append(s)
                m = functools.reduce(jnp.maximum, ls)
                ps = [jnp.exp2(l - m) for l in ls]
                den = functools.reduce(lambda a, b: a + b, ps)
                inv = pl.reciprocal(den, approx=True)
                st["p", i, b, u] = (ps, inv * (2.0 - den * inv) * g_s[pl.ds(r0, 8), :])
            return st["p", i, b, u]

        def pv(i, b, u2, j):
            halves = []
            for u in (2 * u2, 2 * u2 + 1):
                r0 = i * T + RB * b + 8 * u
                ps, inv = probs(i, b, u)
                o = None
                for w in range(W):
                    t = ps[w] * v_s[j, pl.ds(HALO + r0 - DIL * w, 8), :]
                    o = t if o is None else o + t
                halves.append(o * inv)
            r0 = i * T + RB * b + 16 * u2
            o = jnp.concatenate(halves, axis=0).astype(BF16)
            o_s[pl.ds(r0 // 2, 8), pl.ds(128 * j, 128)] = pltpu.bitcast(o, U32)
            add_dep(o)

        def outproj(i, j0, nw):
            lhs = pltpu.bitcast(tie(o_s[pl.ds(i * T // 2, T // 2), :]), BF16)
            rhs = pltpu.bitcast(wu32[3, :, pl.ds(128 * j0, 128 * nw)], BF16)
            a = jnp.dot(lhs, rhs, preferred_element_type=F32)
            st["res"][st["n"]] = [a[z:z + 8, :128] for z in range(0, T, T // 4)]
            cols = pl.ds(128 * j0, 128 * nw)
            out_v[pl.ds(i * T, T), cols] = (a + y_s[pl.ds(i * T, T), cols]).astype(BF16)

        def residual(i, b):
            r0 = i * T + 16 * b
            og = 1.0 - g_s[pl.ds(r0, 16), :]
            xb = pltpu.bitcast(xu[pl.ds(r0 // 2, 8), :], BF16).astype(F32)
            for j in range(NJ):
                yb = og * xb[:, 128 * j:128 * (j + 1)]
                y_s[pl.ds(r0, 16), pl.ds(128 * j, 128)] = yb
            add_dep(yb[8:])

        int_min = np.int32(-2 ** 31)

        def top_stage(n):
            if n == 0:
                keys = []
                for c, r in enumerate(st["racc"]):
                    r = r.astype(BF16).astype(F32)
                    r = jnp.where(r != r, -jnp.inf, jnp.where(r == 0.0, 0.0, r))
                    bits = pltpu.bitcast(r, jnp.int32)
                    bits = jnp.where(bits < 0, bits ^ 0x7FFFFFFF, bits)
                    keys.append((bits & -65536) | (S - 1 - ((sub + 8 * c) * 128 + lane)))
                st["keys"], st["top"] = keys, []
            m = functools.reduce(jnp.maximum, st["keys"])
            m = jnp.max(jnp.max(m, axis=0, keepdims=True), axis=1, keepdims=True)
            st["keys"] = [jnp.where(k == m, int_min, k) for k in st["keys"]]
            st["top"].append(m)
            add_dep(*st["keys"])

        def gather_rows():
            row16 = _iota((16, D), 0)
            xs = jnp.zeros((16, D), F32)
            st["sel"] = []
            for n, m in enumerate(st["top"]):
                hi = m & -65536
                score = pltpu.bitcast(jnp.where(hi < 0, (hi | 0xFFFF) ^ 0x7FFFFFFF, hi), F32)
                idx = S - 1 - (m[0, 0] & 0xFFFF)
                st["sel"].append((idx, score))
                base = pl.multiple_of(jnp.clip((idx // 16) * 16, 0, S - 16), 16)
                blk = x_v[pl.ds(base, 16), :].astype(F32)
                xr = jnp.sum(jnp.where(row16 + base == idx, blk, 0.0), axis=0, keepdims=True)
                xs = jnp.where(row16 == n, xr, xs)
            st["xs"] = xs.astype(BF16)

        def acc(key, val):
            st[key] = val if key not in st else st[key] + val

        def ffn_tile(kind, n, k):
            f0 = 128 * n
            rows, cols = pl.ds(f0, min(128, F - f0)), pl.ds(128 * k, 128)
            if kind < 2:
                wt = (wg_v, wu_v)[kind][rows, cols]
                acc(("h", kind, n), jax.lax.dot_general(st["xs"][:, 128 * k:128 * (k + 1)], wt, NT_DIMS, preferred_element_type=F32))
                if kind == 1 and k == NJ - 1:
                    hg, hu = st.pop(("h", 0, n)), st.pop(("h", 1, n))
                    st["hh", n] = (hg * jax.nn.sigmoid(hg) * hu).astype(BF16)
            else:
                acc(("y", k), jnp.dot(st["hh", n], wd_v[rows, cols], preferred_element_type=F32))

        def patch(lo, hi, js=range(NJ)):
            row16 = _iota((16, 128), 0)
            for n, (idx, m) in enumerate(st["sel"]):
                rs = jax.nn.sigmoid(m)
                base = pl.multiple_of(jnp.clip((idx // 16) * 16, lo, hi - 16), 16)
                og = 1.0 - g_s[pl.ds(base, 16), :]
                hit = row16 + base == idx
                for j in js:
                    cur = out_v[pl.ds(base, 16), pl.ds(128 * j, 128)].astype(F32)
                    new = jnp.where(hit, cur + og * (st["y", j][n:n + 1] * rs), cur)
                    out_v[pl.ds(base, 16), pl.ds(128 * j, 128)] = new.astype(BF16)

        groups = [(j0, min(NW, NJ - j0)) for j0 in range(0, NJ, NW)]
        mxu = []
        na = nc = 0
        for ch in order:
            if ch == "A":
                mxu += [("A", na, p, j0, nw) for p in (1, 2, 0) for j0, nw in groups]
                na += 1
            else:
                mxu += [("C", nc, 3, j0, nw) for j0, nw in groups]
                nc += 1
        assert na == NT and nc == NT
        mxu[:len(head) // 2 * len(groups)] = [("A", int(head[z + 1]), "QKV".index(head[z]), j0, nw) for z in range(0, len(head), 2) for j0, nw in groups]
        pos, t = [], 0
        for m_ in mxu:
            pos.append(t)
            t += m_[4]
        total = t
        a_done = {i: max(pos[n] + m_[4] for n, m_ in enumerate(mxu) if m_[0] == "A" and m_[1] == i) for i in range(NT)}
        c_start = {i: min(pos[n] for n, m_ in enumerate(mxu) if m_[0] == "C" and m_[1] == i) for i in range(NT)}
        b0 = a_done[0]
        b1 = c_start[NT - 1] if b_end is None else b_end
        vq = []

        def xdue(i, b):
            if i == 0:
                return 0
            if i == 1:
                return min(pos[n] for n, m_ in enumerate(mxu) if m_[:2] == ("A", 1)) - x1lag + 0.05 * b / G
            if i == 2:
                return 24 + 4 * b / G
            return x_at + x_span * ((i - 3) * G + b) / ((NT - 3) * G)

        for i in range(NT):
            for b in range(G):
                due = b0 + (b1 - b0) * (i * G + b) / (NT * G)
                due = max(due, a_done[i] + lag - 1)
                if do_attn and (16 * b) % RB == 0:
                    span = (b1 - b0) * RB / S
                    due = max(min(due, c_start[i] - pvlag - span * (G - b) * 16 / RB), a_done[i])
                    vq.append((due, 1, ("QK", i, 16 * b // RB)))
                    if b == 0:
                        vq.append((due + pvlag - glag, 0, ("G", i)))
                    nsub = (RB // 16) * (NJ + 2)
                    for u2 in range(RB // 16):
                        vq.append((min(due + pvlag, c_start[i]), 0.4, ("Y", i, b + u2)))
                        for z in range(NJ + 2):
                            t_sub = min(due + pvlag + span * (u2 * (NJ + 2) + z) / nsub, c_start[i])
                            if z < 2:
                                vq.append((t_sub, 0.5, ("SM", i, 16 * b // RB, 2 * u2 + z)))
                            else:
                                vq.append((t_sub, 0.5, ("PV", i, 16 * b // RB, u2, z - 2)))
                if i >= 1:
                    vq.append((xdue(i, b), -1, ("X", i, b)))
        for n in range(S // 128):
            i = n * 128 // T
            vq.append((max(r_from + n * r_every, np.ceil(xdue(i, G - 1)) + 1), 0, ("R", n)))
        r_to = max(e[0] for e in vq if e[2][0] == "R")
        for r in range(D // 16):
            vq.append((hold[0] + 0.5 + r / 1000, -2, ("W", 2, r)))
            vq.append((hold[1] + 0.6 + r / 1000, -2, ("W", 0, r)))
        wo_at = c_start[0] - 8 - wo_span
        for t_ in range(NJ):
            for c in range(D // 64):
                vq.append((wo_at + (t_ * 10 + c) / 8, -2, ("WF", t_, c)))
            for j in range(NJ):
                for c in range(4):
                    vq.append((wo_at + 7 + wo_span * (t_ * 20 + j * 4 + c) / 100, -2, ("WO", t_, j, c)))
        if do_ffn:
            for n in range(CAP):
                vq.append((r_to + 2.5 + n, 2, ("T", n)))
            assert r_to + 2.5 + CAP <= ffn_at - 1
            vq.append((ffn_at - 1, 2, ("S",)))
            nf = -(-F // 128)
            seq = []
            for n in range(nf):
                seq += [(0, n), (1, n)]
                if n >= 2:
                    seq.append((2, n - 2))
            seq += [(2, nf - 2), (2, nf - 1)]
            seq = [kn + (k,) for kn in seq for k in range(NJ)]
            for n, kn in enumerate(seq):
                vq.append((ffn_at + n // ffn_per, 3 + n / 1000, ("F",) + kn))
            ffn_done = ffn_at + len(seq) // ffn_per + 1
        else:
            ffn_done = 0
        vq.sort(key=lambda e: (e[0], e[1]))

        waited = set()

        def need(name, cp):
            if name not in waited:
                waited.add(name)
                cp.wait()

        def emit(item):
            k = item[0]
            if k == "QK":
                qk(item[1], item[2])
            elif k == "PV":
                pv(*item[1:])
            elif k == "SM":
                add_dep(probs(*item[1:])[1])
            elif k == "R":
                need("wr", wr_cp); need("gw", gw_cp)
                if 'r' not in abl:
                    router(item[1])
            elif k == "Y":
                residual(item[1], item[2])
            elif k == "G":
                gate(item[1])
            elif k == "X":
                if item[1] == 1:
                    need(("x", 1), x_cp[1])
                elif item[1] > 2 and ("x", 3) not in waited:
                    need(("x", 3), x_cp[3]); need("wo", wo_cp)
                    wg_cp.start(); wu_cp.start(); wd_cp.start()
                pack_x(item[1], item[2])
            elif k == "W":
                if item[1] == 1:
                    c = 16 * item[2] // WC
                    if ("wk", c) not in waited:
                        waited.add(("wk", c))
                        if c == 0:
                            pass
                elif ("w", item[1]) not in waited:
                    need(("w", item[1]), w_cp[item[1] // 2])
                    if item[1] == 2:
                        w_cp[0].start(); x_cp[2].start(); wr_cp.start(); gw_cp.start()
                    else:
                        need(("x", 2), x_cp[2]); need("wr", wr_cp); need("gw", gw_cp)
                        x_cp[3].start(); wo_cp.start()
                if 'w' not in abl:
                    permute_w(item[1], item[2])
            elif k == "WF":
                need("wo", wo_cp)
                widen_wo(item[1], item[2])
            elif k == "WO":
                permute_wo(*item[1:])
            elif k == "T":
                top_stage(item[1])
            elif k == "S":
                need("wg", wg_cp); need("wu", wu_cp); need("wd", wd_cp)
                gather_rows()
            elif k == "F":
                ffn_tile(*item[1:])

        for c in range(NWC):
            wk_cp[c].start()
        for j in range(NJ):
            k_s[j, pl.ds(0, HALO), :] = jnp.zeros((HALO, 128), F32)
        import contextlib
        sc = (lambda n: jax.named_scope("u9%02d" % n)) if prof else (lambda n: contextlib.nullcontext())
        for c in range(NWC):
            with sc(2 * c):
                need(("wk0", c), wk_cp[c])
                if c == 0:
                    x_cp[0].start()
                if c == NWC - 1:
                    x_cp[1].start(); w_cp[1].start()
            with sc(2 * c + 1):
                for r in range(c * WC // 16, (c + 1) * WC // 16):
                    emit(("W", 1, r))
        with sc(50):
            need(("x", 0), x_cp[0])
        with sc(51):
            for b in range(G):
                pack_x(0, b)
        st["dep"] = {}
        u0 = xu[pl.ds(0, 8), pl.ds(0, 128)]
        st["true"] = ((u0 & 1) + ((~u0) & 1)) == 1

        def soft(item, m_):
            return item[0] in ("SM", "PV", "WF", "WO", "X", "T", "Y") and not (m_[0] == "C" and m_[1] == item[1])

        qi = 0
        sent = 0
        csent = 0
        outs = []
        scope = None
        for n, m_ in enumerate(mxu):
            if prof and n % prof == 0:
                if scope is not None:
                    scope.__exit__(None, None, None)
                scope = jax.named_scope("u%03d" % n)
                scope.__enter__()
            while qi < len(vq) and vq[qi][0] <= pos[n] + (m_[4] * (NJ - 1) / NJ if soft(vq[qi][2], m_) else 0):
                st["slot"] = min(NJ - 1, max(0, int(np.ceil((vq[qi][0] - pos[n]) * NJ / m_[4] - 1e-9))))
                emit(vq[qi][2]); qi += 1
            st["n"] = n
            if m_[0] == "A":
                proj(m_[1], m_[2], m_[3], m_[4])
            else:
                outproj(m_[1], m_[3], m_[4])
                if m_[1] == NT - 1:
                    assert sent == NT - 1
                    if m_[3] + m_[4] in col_cuts:
                        js = range(csent, m_[3] + m_[4])
                        csent = m_[3] + m_[4]
                        patch(m_[1] * T, m_[1] * T + T, js)
                        outs.append(o_copy(m_[1], m_[1] + 1, js[0], csent, len(outs)))
                        outs[-1].start()
                elif m_[3] + m_[4] == NJ and m_[1] + 1 in row_cuts:
                    assert pos[n] >= ffn_done
                    patch(sent * T, (m_[1] + 1) * T)
                    outs.append(o_copy(sent, m_[1] + 1, 0, NJ, len(outs)))
                    outs[-1].start()
                    sent = m_[1] + 1
        assert qi == len(vq)
        if scope is not None:
            scope.__exit__(None, None, None)
        if not do_ffn and 'f' not in abl:
            wg_cp.wait(); wu_cp.wait(); wd_cp.wait()
        for cp in outs:
            cp.wait()

    hbm = pl.BlockSpec(memory_space=pltpu.HBM)

    @jax.jit
    def fn(A_x, A_wqkv, A_wo, B_x, B_w_r, B_w_gate, B_w_up, B_w_down, gate_w):
        return pl.pallas_call(
            kernel,
            out_shape=jax.ShapeDtypeStruct((1, S, D), BF16),
            in_specs=[hbm] * 8,
            out_specs=hbm,
            scratch_shapes=[
                pltpu.VMEM((S + 3 * F, D), BF16), pltpu.VMEM((4, D, D), BF16), pltpu.VMEM((D, D), BF16),
                pltpu.VMEM((NJ, D + 8, 128), F32),
                pltpu.VMEM((S // 2, D), U32), pltpu.VMEM((4, D // 2, D), U32),
                pltpu.VMEM((NJ, S, 128), F32), pltpu.VMEM((NJ, S + HALO, 128), F32), pltpu.VMEM((NJ, S + HALO, 128), F32),
                pltpu.VMEM((S // 2, D), U32), pltpu.VMEM((S, 128), F32), pltpu.VMEM((S, D), F32), pltpu.VMEM((S, D), BF16),
                pltpu.VMEM((D,), BF16), pltpu.VMEM((D,), BF16),
                pltpu.SemaphoreType.DMA((NT + 9,)), pltpu.SemaphoreType.DMA((NWC,)), pltpu.SemaphoreType.DMA((len(row_cuts) + len(col_cuts),)),
            ],
            compiler_params=pltpu.CompilerParams(vmem_limit_bytes=100 * 1024 * 1024, flags=flags),
        )(A_x, A_wqkv, A_wo, B_w_r, B_w_gate.T, B_w_up.T, B_w_down, gate_w)
    return fn


_fn = make()


@jax.jit
def pallas_gated_mix__sliding_local_dilated__moe_arch_mod__prompt_kernel(
    A_x, A_wqkv, A_wo, B_x, B_w_r, B_w_gate, B_w_up, B_w_down, gate_w):
    return _fn(A_x, A_wqkv, A_wo, B_x, B_w_r, B_w_gate, B_w_up, B_w_down, gate_w)
```

```python
import functools
import numpy as np
import jax
import jax.numpy as jnp
import jax.experimental.pallas as pl
import jax.experimental.pallas.tpu as pltpu

S, D, F = 2048, 640, 1728
H, DH, W, DIL, CAP = 32, 20, 8, 2, 2
NJ = D // 128
HALO = 16
LOG2E = 1.4426950408889634
F32, BF16, U32 = jnp.float32, jnp.bfloat16, jnp.uint32
NT_DIMS = (((1,), (1,)), ((), ()))


def _iota(shape, dim):
    return jax.lax.broadcasted_iota(jnp.int32, shape, dim)


T = 256
NT, G = S // T, T // 16
KS = 256
ORDER = "AAAAACCAAACCCCCC"
HEAD = "K0K1V0V1Q0Q1"
HOLD = (7, 15)
X_AT, X_SPAN = 38, 28
R_FROM, R_EVERY = 17, 3
WO_SPAN = 20
FFN_AT, FFN_PER = 78, 4
PV_LAG, Q_LEAD = 3, 2
ROW_CUTS = (4, 5, 6, 7)


def _kernel(x_hbm, wqkv_hbm, wo_hbm, wr_hbm, wg_hbm, wu_hbm, wd_hbm, gw_hbm, out_hbm,
            big, w_v, wo_v, wo_f, xu, wu32, q_s, k_s, v_s, o_s, g_s, y_s, out_v, wr_v, gw_v, sem, wsem, osem):
    x_v = big.at[pl.ds(0, S)]
    wg_v, wu_v, wd_v = (big.at[pl.ds(S + n * F, F)] for n in range(3))
    x_cp = [pltpu.make_async_copy(x_hbm.at[0, pl.ds(a, n)], x_v.at[pl.ds(a, n)], sem.at[i])
            for i, (a, n) in enumerate(((0, T), (T, T), (2 * T, T), (3 * T, S - 3 * T)))]
    wk_cp = [pltpu.make_async_copy(wqkv_hbm.at[pl.ds(a, n), pl.ds(D, D)], w_v.at[1, pl.ds(a, n)], wsem.at[c])
             for c, (a, n) in enumerate(((0, KS), (KS, D - KS)))]
    w_cp = [pltpu.make_async_copy(wqkv_hbm.at[:, pl.ds(p * D, D)], w_v.at[p], sem.at[NT + p]) for p in (0, 2)]
    wo_cp = pltpu.make_async_copy(wo_hbm, wo_v, sem.at[NT + 3])
    wg_cp = pltpu.make_async_copy(wg_hbm, wg_v, sem.at[NT + 4])
    wu_cp = pltpu.make_async_copy(wu_hbm, wu_v, sem.at[NT + 5])
    wd_cp = pltpu.make_async_copy(wd_hbm, wd_v, sem.at[NT + 6])
    wr_cp = pltpu.make_async_copy(wr_hbm, wr_v, sem.at[NT + 7])
    gw_cp = pltpu.make_async_copy(gw_hbm, gw_v, sem.at[NT + 8])

    def o_copy(i0, i1, j0, j1, n):
        rows, cols = pl.ds(i0 * T, (i1 - i0) * T), pl.ds(128 * j0, 128 * (j1 - j0))
        return pltpu.make_async_copy(out_v.at[rows, cols], out_hbm.at[0, rows, cols], osem.at[n])

    lane = _iota((8, 128), 1)
    st = dict(racc=[jnp.zeros((8, 128), F32) for _ in range(S // 1024)], dep={}, res={}, n=-1, slot=0, true=None)

    def add_dep(*vals):
        k = st["slot"]
        for v in vals:
            v = pltpu.bitcast(v, U32)
            st["dep"][k] = v if st["dep"].get(k) is None else st["dep"][k] | v

    def tie(lhs):
        d, st["dep"] = st["dep"], {}
        if not d:
            return lhs
        top = [lhs[:8, 128 * k:128 * (k + 1)] for k in range(NJ)]
        top = [jnp.where(st["true"], t, d[k]) if k in d else t for k, t in enumerate(top)]
        return jnp.concatenate([jnp.concatenate(top, axis=1), lhs[8:]], axis=0)

    def permute_w(p, r):
        src = [pltpu.bitcast(w_v[p, pl.ds(16 * r, 16), pl.ds(128 * t, 128)], U32) for t in range(NJ)]
        for j in range(NJ):
            m = src[0]
            for t in range(1, NJ):
                m = jnp.where((128 * t + lane) % 5 == j, src[t], m)
            if j:
                m = pltpu.roll(m, 128 - j, 1)
            wu32[p, pl.ds(8 * r, 8), pl.ds(128 * j, 128)] = m

    def widen_wo(t, c):
        blk = wo_v[pl.ds(64 * c, 64), pl.ds(128 * t, 128)].astype(F32)
        wo_f[t, pl.ds(64 * c, 64), :] = blk
        if c == 0:
            wo_f[t, pl.ds(D, 8), :] = jnp.zeros((8, 128), F32)
        add_dep(blk[56:])

    def permute_wo(t, j, c):
        outs = []
        for m0 in range(32 * c, 32 * c + 32, 8):
            tile = (3 * (_iota((8, 128), 0) + m0)) % 5
            blk = wo_f[t, pl.ds(m0 + j, 8), :]
            for z in range(1, NJ):
                blk = jnp.where(tile == z, wo_f[t, pl.ds(128 * z + m0 + j, 8), :], blk)
            outs.append(blk)
        blk = pltpu.bitcast(jnp.concatenate(outs, axis=0).astype(BF16), U32)
        wu32[3, pl.ds(64 * j + 16 * c, 16), pl.ds(128 * t, 128)] = blk
        add_dep(blk[:8], blk[8:])

    def pack_x(i, b):
        r0 = i * T + 16 * b
        blk = pltpu.bitcast(x_v[pl.ds(r0, 16), :], U32)
        xu[pl.ds(r0 // 2, 8), :] = blk
        add_dep(blk[:, D - 128:])

    def proj(i, p, j0):
        dst, off = ((q_s, 0), (k_s, HALO), (v_s, HALO))[p]
        k0 = KS if (i, p) == (0, 1) else 0
        lhs = pltpu.bitcast(tie(xu[pl.ds(i * T // 2, T // 2), :])[:, k0:], BF16)
        rhs = pltpu.bitcast(wu32[p, pl.ds(k0 // 2, (D - k0) // 2), pl.ds(128 * j0, 128)], BF16)
        r = jnp.dot(lhs, rhs, preferred_element_type=F32)
        if k0:
            r = r + k_s[j0, pl.ds(HALO, T), :]
        st["res"][st["n"]] = [r[z:z + 8, :128] for z in range(0, T, T // 4)]
        if st["n"] in HOLD:
            w_v[3, pl.ds(0, 16), pl.ds(0, 128)] = r[:16, :128].astype(BF16)
        dst[j0, pl.ds(off + i * T, T), :] = r
        if i == 0 and p == 2:
            v_s[j0, pl.ds(0, HALO), :] = jnp.broadcast_to(r[0:1], (HALO, 128))

    sub = _iota((8, 128), 0)

    def router(i):
        if "wrg" not in st:
            wr = jnp.broadcast_to(wr_v[...].astype(F32).reshape(1, D), (8, D))
            gw = jnp.broadcast_to(gw_v[...].astype(F32).reshape(1, D), (8, D))
            st["wrg"] = jnp.concatenate([wr, gw], axis=0).astype(BF16)
        xt = pltpu.bitcast(xu[pl.ds(64 * i, 64), :], BF16)
        rg = jax.lax.dot_general(st["wrg"], xt, NT_DIMS, preferred_element_type=F32)
        st["racc"][i // 8] = jnp.where(sub == i % 8, rg[:8], st["racc"][i // 8])
        st["g", i] = jax.nn.sigmoid(rg[8:])

    def gate(i):
        diag = [jnp.where(lane == sub + 8 * u, st["g", n], 0.0)
                for n in range(i * T // 128, (i + 1) * T // 128) for u in range(16)]
        diag = jnp.concatenate(diag, axis=0).astype(BF16)
        g_s[pl.ds(i * T, T), :] = jnp.dot(diag, jnp.ones((128, 128), BF16), preferred_element_type=F32)

    cs = (DH ** -0.5) * LOG2E

    rmat = jnp.where((77 * _iota((128, 128), 0)) % 128 // 4 == (77 * _iota((128, 128), 1)) % 128 // 4,
                     1.0, 0.0).astype(BF16)

    def qk(i, b):
        r0 = i * T + 16 * b
        parts = [[None, None] for _ in range(W)]
        for u in range(2):
            q = [q_s[j, pl.ds(r0 + 8 * u, 8), :] for j in range(NJ)]
            recent = st["res"].get(st["n"] + 1 - Q_LEAD)
            csv = cs if recent is None else jnp.where(st["true"], cs, recent[2 * u])
            q = [qq * csv for qq in q]
            for w in range(W):
                acc_w = None
                for j in range(NJ):
                    t = q[j] * k_s[j, pl.ds(HALO + r0 + 8 * u - DIL * w, 8), :]
                    acc_w = t if acc_w is None else acc_w + t
                parts[w][u] = acc_w
        cat = jnp.concatenate([p for pw in parts for p in pw], axis=0).astype(BF16)
        st["l", i, b] = jnp.dot(cat, rmat, preferred_element_type=F32)

    def probs(i, b, u):
        if ("p", i, b, u) not in st:
            lg = st["l", i, b]
            r0 = i * T + 16 * b + 8 * u
            ls = []
            for w in range(W):
                s = lg[w * 16 + 8 * u:w * 16 + 8 * u + 8]
                if r0 < DIL * w:
                    s = jnp.where(_iota((8, 128), 0) + r0 >= DIL * w, s, -1e9 * LOG2E)
                ls.append(s)
            m = functools.reduce(jnp.maximum, ls)
            ps = [jnp.exp2(l - m) for l in ls]
            den = functools.reduce(lambda a, b: a + b, ps)
            inv = pl.reciprocal(den, approx=True)
            st["p", i, b, u] = (ps, inv * (2.0 - den * inv) * g_s[pl.ds(r0, 8), :])
        return st["p", i, b, u]

    def pv(i, b, j):
        halves = []
        for u in range(2):
            r0 = i * T + 16 * b + 8 * u
            ps, inv = probs(i, b, u)
            o = None
            for w in range(W):
                t = ps[w] * v_s[j, pl.ds(HALO + r0 - DIL * w, 8), :]
                o = t if o is None else o + t
            halves.append(o * inv)
        r0 = i * T + 16 * b
        o = jnp.concatenate(halves, axis=0).astype(BF16)
        o_s[pl.ds(r0 // 2, 8), pl.ds(128 * j, 128)] = pltpu.bitcast(o, U32)
        add_dep(o)

    def outproj(i, j0):
        lhs = pltpu.bitcast(tie(o_s[pl.ds(i * T // 2, T // 2), :]), BF16)
        rhs = pltpu.bitcast(wu32[3, :, pl.ds(128 * j0, 128)], BF16)
        a = jnp.dot(lhs, rhs, preferred_element_type=F32)
        st["res"][st["n"]] = [a[z:z + 8, :128] for z in range(0, T, T // 4)]
        cols = pl.ds(128 * j0, 128)
        out_v[pl.ds(i * T, T), cols] = (a + y_s[pl.ds(i * T, T), cols]).astype(BF16)

    def residual(i, b):
        r0 = i * T + 16 * b
        og = 1.0 - g_s[pl.ds(r0, 16), :]
        xb = pltpu.bitcast(xu[pl.ds(r0 // 2, 8), :], BF16).astype(F32)
        for j in range(NJ):
            yb = og * xb[:, 128 * j:128 * (j + 1)]
            y_s[pl.ds(r0, 16), pl.ds(128 * j, 128)] = yb
        add_dep(yb[8:])

    int_min = np.int32(-2 ** 31)

    def top_stage(n):
        if n == 0:
            keys = []
            for c, r in enumerate(st["racc"]):
                r = r.astype(BF16).astype(F32)
                r = jnp.where(r != r, -jnp.inf, jnp.where(r == 0.0, 0.0, r))
                bits = pltpu.bitcast(r, jnp.int32)
                bits = jnp.where(bits < 0, bits ^ 0x7FFFFFFF, bits)
                keys.append((bits & -65536) | (S - 1 - ((sub + 8 * c) * 128 + lane)))
            st["keys"], st["top"] = keys, []
        m = functools.reduce(jnp.maximum, st["keys"])
        m = jnp.max(jnp.max(m, axis=0, keepdims=True), axis=1, keepdims=True)
        st["keys"] = [jnp.where(k == m, int_min, k) for k in st["keys"]]
        st["top"].append(m)
        add_dep(*st["keys"])

    def gather_rows():
        row16 = _iota((16, D), 0)
        xs = jnp.zeros((16, D), F32)
        st["sel"] = []
        for n, m in enumerate(st["top"]):
            hi = m & -65536
            score = pltpu.bitcast(jnp.where(hi < 0, (hi | 0xFFFF) ^ 0x7FFFFFFF, hi), F32)
            idx = S - 1 - (m[0, 0] & 0xFFFF)
            st["sel"].append((idx, score))
            base = pl.multiple_of(jnp.clip((idx // 16) * 16, 0, S - 16), 16)
            blk = x_v[pl.ds(base, 16), :].astype(F32)
            xr = jnp.sum(jnp.where(row16 + base == idx, blk, 0.0), axis=0, keepdims=True)
            xs = jnp.where(row16 == n, xr, xs)
        st["xs"] = xs.astype(BF16)

    def acc(key, val):
        st[key] = val if key not in st else st[key] + val

    def ffn_tile(kind, n, k):
        f0 = 128 * n
        rows, cols = pl.ds(f0, min(128, F - f0)), pl.ds(128 * k, 128)
        if kind < 2:
            wt = (wg_v, wu_v)[kind][rows, cols]
            acc(("h", kind, n), jax.lax.dot_general(st["xs"][:, 128 * k:128 * (k + 1)], wt, NT_DIMS, preferred_element_type=F32))
            if kind == 1 and k == NJ - 1:
                hg, hu = st.pop(("h", 0, n)), st.pop(("h", 1, n))
                st["hh", n] = (hg * jax.nn.sigmoid(hg) * hu).astype(BF16)
        else:
            acc(("y", k), jnp.dot(st["hh", n], wd_v[rows, cols], preferred_element_type=F32))

    def patch(lo, hi, js=range(NJ)):
        row16 = _iota((16, 128), 0)
        for n, (idx, m) in enumerate(st["sel"]):
            rs = jax.nn.sigmoid(m)
            base = pl.multiple_of(jnp.clip((idx // 16) * 16, lo, hi - 16), 16)
            og = 1.0 - g_s[pl.ds(base, 16), :]
            hit = row16 + base == idx
            for j in js:
                cur = out_v[pl.ds(base, 16), pl.ds(128 * j, 128)].astype(F32)
                new = jnp.where(hit, cur + og * (st["y", j][n:n + 1] * rs), cur)
                out_v[pl.ds(base, 16), pl.ds(128 * j, 128)] = new.astype(BF16)

    mxu, na, nc = [], 0, 0
    for ch in ORDER:
        if ch == "A":
            mxu += [("A", na, p, j) for p in (1, 2, 0) for j in range(NJ)]
            na += 1
        else:
            mxu += [("C", nc, 3, j) for j in range(NJ)]
            nc += 1
    assert na == NT and nc == NT
    mxu[:len(HEAD) // 2 * NJ] = [("A", int(HEAD[z + 1]), "QKV".index(HEAD[z]), j)
                                 for z in range(0, len(HEAD), 2) for j in range(NJ)]
    a_start = {i: min(n for n, m_ in enumerate(mxu) if m_[:2] == ("A", i)) for i in range(NT)}
    a_done = {i: max(n + 1 for n, m_ in enumerate(mxu) if m_[:2] == ("A", i)) for i in range(NT)}
    c_start = {i: min(n for n, m_ in enumerate(mxu) if m_[:2] == ("C", i)) for i in range(NT)}

    def xdue(i, b):
        if i == 0:
            return 0
        if i == 1:
            return a_start[1] - 1.1 + 0.05 * b / G
        if i == 2:
            return 24 + 4 * b / G
        return X_AT + X_SPAN * ((i - 3) * G + b) / ((NT - 3) * G)

    vq = []
    b0, b1 = a_done[0], c_start[NT - 1]
    span = (b1 - b0) * 16 / S
    for i in range(NT):
        for b in range(G):
            due = max(b0 + (b1 - b0) * (i * G + b) / (NT * G), a_done[i])
            due = max(min(due, c_start[i] - PV_LAG - span * (G - b)), a_done[i])
            vq.append((due, 1, ("QK", i, b)))
            if b == 0:
                vq.append((due + PV_LAG - 1, 0, ("G", i)))
            vq.append((min(due + PV_LAG, c_start[i]), 0.4, ("Y", i, b)))
            for z in range(NJ + 2):
                t_sub = min(due + PV_LAG + span * z / (NJ + 2), c_start[i])
                vq.append((t_sub, 0.5, ("SM", i, b, z) if z < 2 else ("PV", i, b, z - 2)))
            if i >= 1:
                assert xdue(i, b) <= a_start[i]
                vq.append((xdue(i, b), -1, ("X", i, b)))
    for n in range(S // 128):
        vq.append((max(R_FROM + n * R_EVERY, np.ceil(xdue(n * 128 // T, G - 1)) + 1), 0, ("R", n)))
    r_to = max(e[0] for e in vq if e[2][0] == "R")
    for r in range(D // 16):
        vq.append((HOLD[0] + 0.5 + r / 1000, -2, ("W", 2, r)))
        vq.append((HOLD[1] + 0.6 + r / 1000, -2, ("W", 0, r)))
    wo_at = c_start[0] - 8 - WO_SPAN
    assert HOLD[0] + 1 <= mxu.index(("A", 0, 2, 0)) and HOLD[1] + 1 <= mxu.index(("A", 0, 0, 0)) <= R_FROM + 3
    for t_ in range(NJ):
        for c in range(D // 64):
            vq.append((wo_at + (t_ * 10 + c) / 8, -2, ("WF", t_, c)))
        for j in range(NJ):
            for c in range(4):
                vq.append((wo_at + 7 + WO_SPAN * (t_ * 20 + j * 4 + c) / 100, -2, ("WO", t_, j, c)))
    for n in range(CAP):
        vq.append((r_to + 2.5 + n, 2, ("T", n)))
    assert r_to + 2.5 + CAP <= FFN_AT - 1
    vq.append((FFN_AT - 1, 2, ("S",)))
    nf = -(-F // 128)
    seq = []
    for n in range(nf):
        seq += [(0, n), (1, n)]
        if n >= 2:
            seq.append((2, n - 2))
    seq += [(2, nf - 2), (2, nf - 1)]
    seq = [kn + (k,) for kn in seq for k in range(NJ)]
    for n, kn in enumerate(seq):
        vq.append((FFN_AT + n // FFN_PER, 3 + n / 1000, ("F",) + kn))
    ffn_done = FFN_AT + len(seq) // FFN_PER + 1
    vq.sort(key=lambda e: (e[0], e[1]))

    waited = set()

    def need(name, cp):
        if name not in waited:
            waited.add(name)
            cp.wait()

    def emit(item):
        k = item[0]
        if k == "QK":
            qk(item[1], item[2])
        elif k == "PV":
            pv(*item[1:])
        elif k == "SM":
            add_dep(probs(*item[1:])[1])
        elif k == "R":
            need("wr", wr_cp); need("gw", gw_cp)
            router(item[1])
        elif k == "Y":
            residual(item[1], item[2])
        elif k == "G":
            gate(item[1])
        elif k == "X":
            if item[1] == 1:
                need(("x", 1), x_cp[1])
            elif item[1] > 2 and ("x", 3) not in waited:
                need(("x", 3), x_cp[3]); need("wo", wo_cp)
                wg_cp.start(); wu_cp.start(); wd_cp.start()
            pack_x(item[1], item[2])
        elif k == "W":
            if ("w", item[1]) not in waited:
                need(("w", item[1]), w_cp[item[1] // 2])
                if item[1] == 2:
                    w_cp[0].start(); x_cp[2].start(); wr_cp.start(); gw_cp.start()
                else:
                    need(("x", 2), x_cp[2]); need("wr", wr_cp); need("gw", gw_cp)
                    x_cp[3].start(); wo_cp.start()
            permute_w(item[1], item[2])
        elif k == "WF":
            need("wo", wo_cp)
            widen_wo(item[1], item[2])
        elif k == "WO":
            permute_wo(*item[1:])
        elif k == "T":
            top_stage(item[1])
        elif k == "S":
            need("wg", wg_cp); need("wu", wu_cp); need("wd", wd_cp)
            gather_rows()
        elif k == "F":
            ffn_tile(*item[1:])

    x_cp[0].start(); wk_cp[0].start()
    for j in range(NJ):
        k_s[j, pl.ds(0, HALO), :] = jnp.zeros((HALO, 128), F32)
    x_cp[0].wait()
    wk_cp[1].start()
    for b in range(G):
        pack_x(0, b)
    wk_cp[0].wait()
    x_cp[1].start()
    for r in range(KS // 16):
        permute_w(1, r)
    k_head = jnp.dot(pltpu.bitcast(xu[pl.ds(0, T // 2), pl.ds(0, KS)], BF16),
                     pltpu.bitcast(wu32[1, pl.ds(0, KS // 2), :], BF16), preferred_element_type=F32)
    for j in range(NJ):
        k_s[j, pl.ds(HALO, T), :] = k_head[:, 128 * j:128 * (j + 1)]
    w_v[3, pl.ds(0, 16), pl.ds(0, 128)] = k_head[:16, D - 128:].astype(BF16)
    wk_cp[1].wait()
    w_cp[1].start()
    for r in range(KS // 16, D // 16):
        permute_w(1, r)
    st["dep"] = {}
    u0 = xu[pl.ds(0, 8), pl.ds(0, 128)]
    st["true"] = ((u0 & 1) + ((~u0) & 1)) == 1

    def soft(item, m_):
        return item[0] in ("SM", "PV", "WF", "WO", "X", "T", "Y") and not (m_[0] == "C" and m_[1] == item[1])

    qi = sent = 0
    outs = []
    for n, m_ in enumerate(mxu):
        kind, i, p, j = m_
        while qi < len(vq) and vq[qi][0] <= n + ((NJ - 1) / NJ if soft(vq[qi][2], m_) else 0):
            st["slot"] = min(NJ - 1, max(0, int(np.ceil((vq[qi][0] - n) * NJ - 1e-9))))
            emit(vq[qi][2])
            qi += 1
        st["n"] = n
        if kind == "A":
            proj(i, p, j)
            continue
        outproj(i, j)
        if i == NT - 1:
            assert sent == NT - 1
            patch(i * T, i * T + T, [j])
            outs.append(o_copy(i, i + 1, j, j + 1, len(outs)))
            outs[-1].start()
        elif j == NJ - 1 and i + 1 in ROW_CUTS:
            assert n >= ffn_done
            patch(sent * T, (i + 1) * T)
            outs.append(o_copy(sent, i + 1, 0, NJ, len(outs)))
            outs[-1].start()
            sent = i + 1
    assert qi == len(vq)
    for cp in outs:
        cp.wait()


@jax.jit
def pallas_gated_mix__sliding_local_dilated__moe_arch_mod__prompt_kernel(
        A_x, A_wqkv, A_wo, B_x, B_w_r, B_w_gate, B_w_up, B_w_down, gate_w):
    del B_x
    hbm = pl.BlockSpec(memory_space=pltpu.HBM)
    return pl.pallas_call(
            _kernel,
            out_shape=jax.ShapeDtypeStruct((1, S, D), BF16),
            in_specs=[hbm] * 8,
            out_specs=hbm,
            scratch_shapes=[
                pltpu.VMEM((S + 3 * F, D), BF16), pltpu.VMEM((4, D, D), BF16), pltpu.VMEM((D, D), BF16),
                pltpu.VMEM((NJ, D + 8, 128), F32),
                pltpu.VMEM((S // 2, D), U32), pltpu.VMEM((4, D // 2, D), U32),
                pltpu.VMEM((NJ, S, 128), F32), pltpu.VMEM((NJ, S + HALO, 128), F32), pltpu.VMEM((NJ, S + HALO, 128), F32),
                pltpu.VMEM((S // 2, D), U32), pltpu.VMEM((S, 128), F32), pltpu.VMEM((S, D), F32), pltpu.VMEM((S, D), BF16),
                pltpu.VMEM((D,), BF16), pltpu.VMEM((D,), BF16),
                pltpu.SemaphoreType.DMA((NT + 9,)), pltpu.SemaphoreType.DMA((2,)), pltpu.SemaphoreType.DMA((len(ROW_CUTS) + NJ,)),
            ],
            compiler_params=pltpu.CompilerParams(vmem_limit_bytes=100 * 1024 * 1024),
        )(A_x, A_wqkv, A_wo, B_w_r, B_w_gate.T, B_w_up.T, B_w_down, gate_w)
```
